```python
import jax
import jax.numpy as jnp

def _softmax(x, axis=-1):
    return jax.nn.softmax(x, axis=axis)
def _gelu(x):
    return jax.nn.gelu(x, approximate=True)
def _silu(x):
    return jax.nn.silu(x)
def _sigmoid(x):
    return jax.nn.sigmoid(x)
def _layernorm(x, axis=-1, eps=1e-5):
    m = jnp.mean(x, axis=axis, keepdims=True)
    v = jnp.var(x, axis=axis, keepdims=True)
    return (x - m) / jnp.sqrt(v + eps)
def _scatter_add(tgt, idx, src, axis=0):
    return tgt.at[idx].add(src)
def _segment_sum(src, seg, n):
    return jax.ops.segment_sum(src, seg, n)
class _Rng:
    def __init__(self, key):
        self._k = key
    def _next(self):
        self._k, sub = jax.random.split(self._k)
        return sub
    def normal(self, shape):
        return jax.random.normal(self._next(), shape, dtype=jnp.bfloat16)
    def randint(self, lo, hi, shape):
        return jax.random.randint(self._next(), shape, lo, hi, dtype=jnp.int32)
    def uniform(self, shape, lo=0.0, hi=1.0):
        return jax.random.uniform(self._next(), shape, jnp.bfloat16, lo, hi)
    def permutation(self, n):
        return jax.random.permutation(self._next(), n)


kernel_name = 'gated_mix__compressed_kv_cla__sliding_block_cached__decode'

def setup_inputs():
    _rng = _Rng(jax.random.key(int.from_bytes(__import__("os").urandom(4), "little")))
    _w = (lambda a: (lambda t: t.astype(jnp.bfloat16) if jnp.issubdtype(t.dtype, jnp.floating) else t)(jnp.asarray(a)))
    def _A_setup():
        B, H, Sq, Sk, D, M = 8, 32, 1, 4096, 128, 512
        Dc = 4 * D
        return {
            "x": _w((lambda *s: _rng.normal(s) * 0.05)(B, Sq, M)),
            "c_kv": _w((lambda *s: _rng.normal(s) * 0.05)(B, Sk, Dc)),
            "w_q": _w((lambda *s: _rng.normal(s) * 0.05)(M, H, D) * (M ** -0.5)),
            "w_uk": _w((lambda *s: _rng.normal(s) * 0.05)(Dc, H, D) * (Dc ** -0.5)),
            "w_uv": _w((lambda *s: _rng.normal(s) * 0.05)(Dc, H, D) * (Dc ** -0.5)),
            "w_o": _w((lambda *s: _rng.normal(s) * 0.05)(H, D, M) * ((H * D) ** -0.5)),
        }
    _A_in = _A_setup()

    def _B_setup():
        B, Sq, D = 8, 1, 512
        Hq, Hkv, Sk, Dh = 32, 8, 4096, 128
        assert Hq % Hkv == 0, (Hq, Hkv)
        return {
            "x": _w((lambda *s: _rng.normal(s) * 0.05)(B, Sq, D)),
            "k_cache": _w((lambda *s: _rng.normal(s) * 0.05)(B, Hkv, Sk, Dh)),
            "v_cache": _w((lambda *s: _rng.normal(s) * 0.05)(B, Hkv, Sk, Dh)),
            "wq": _w((lambda *s: _rng.normal(s) * 0.05)(D, Hq * Dh) * (D ** -0.5)),
            "wo": _w((lambda *s: _rng.normal(s) * 0.05)(Hq * Dh, D) * ((Hq * Dh) ** -0.5)),
        }
    _B_in = _B_setup()

    return {
        "A_x": _A_in["x"],
        "A_c_kv": _A_in["c_kv"],
        "A_w_q": _A_in["w_q"],
        "A_w_uk": _A_in["w_uk"],
        "A_w_uv": _A_in["w_uv"],
        "A_w_o": _A_in["w_o"],
        "B_x": _B_in["x"],
        "B_k_cache": _B_in["k_cache"],
        "B_v_cache": _B_in["v_cache"],
        "B_wq": _B_in["wq"],
        "B_wo": _B_in["wo"],
        "gate_w": _w((lambda *s: _rng.normal(s) * 0.05)(512)),
    }

def reference(A_x, A_c_kv, A_w_q, A_w_uk, A_w_uv, A_w_o, B_x, B_k_cache, B_v_cache, B_wq, B_wo, gate_w):
    def _A_ref(x, c_kv, w_q, w_uk, w_uv, w_o):
        B, Sq, M = x.shape[0], x.shape[1], x.shape[2]
        Sk = c_kv.shape[1]
        H, D = w_q.shape[1], w_q.shape[2]
        q = jnp.einsum("bqm,mhd->bhqd", x, w_q)
        k = jnp.einsum("bkc,chd->bhkd", c_kv, w_uk)
        v = jnp.einsum("bkc,chd->bhkd", c_kv, w_uv)
        scores = jnp.einsum("bhqd,bhkd->bhqk", q, k) * (D ** -0.5)
        off = Sk - Sq
        qi = jnp.arange(Sq)[:, None]
        kj = jnp.arange(Sk)[None, :]
        cmask = kj <= (qi + off)
        scores = jnp.where(cmask[None, None], scores, -1e9)
        p = _softmax(scores, axis=-1)
        ctx = jnp.einsum("bhqk,bhkd->bhqd", p, v)
        return jnp.einsum("bhqd,hdm->bqm", ctx, w_o)

    def _B_ref(x, k_cache, v_cache, wq, wo):
        B, Sq, D = x.shape
        Hq, Dh = 32, 128
        Hkv, Sk = k_cache.shape[1], k_cache.shape[2]
        W = min(4096, max(256, Sk // 4))
        rep = Hq // Hkv
        q = (lambda x, *d: x.transpose(*d))((x @ wq).reshape(B, Sq, Hq, Dh), 0, 2, 1, 3)
        k = jnp.repeat(k_cache[:, :, Sk - W:, :], rep, axis=1)
        v = jnp.repeat(v_cache[:, :, Sk - W:, :], rep, axis=1)
        scores = jnp.einsum("bhqd,bhkd->bhqk", q, k) * (Dh ** -0.5)
        p = _softmax(scores, axis=-1)
        o = jnp.einsum("bhqk,bhkd->bhqd", p, v)
        return (lambda x, *d: x.transpose(*d))(o, 0, 2, 1, 3).reshape(B, Sq, Hq * Dh) @ wo

    x = A_x
    g = _sigmoid((x * gate_w).sum(-1, keepdims=True))
    a = _A_ref(x, A_c_kv, A_w_q, A_w_uk, A_w_uv, A_w_o)
    b = _B_ref(x, B_k_cache, B_v_cache, B_wq, B_wo)
    return g * a + (1 - g) * b
```

```python
import functools
import math

import jax
import jax.numpy as jnp
from jax import lax
import jax.experimental.pallas as pl
import jax.experimental.pallas.tpu as pltpu

F32 = jnp.float32
BF16 = jnp.bfloat16
U32 = jnp.uint32
NT = (((1,), (1,)), ((), ()))
LOG2E = math.log2(math.e)

NB = 8
SK = 4096
DC = 512
NH = 32
HD = 128
DM = 512
HKV = 8
WIN = 1024

LOOKAHEAD = 2
NSEM = 4
PIECES = 16


def _unpack_pair(w_u32, j):
    u = w_u32[pl.ds(j, 512, stride=16), :]
    lo = pltpu.bitcast(u << 16, F32).astype(BF16)
    hi = pltpu.bitcast(u & jnp.uint32(0xFFFF0000), F32).astype(BF16)
    return lo, hi


def _kernel(x_hbm, ckv_hbm, wq_hbm, wuk_hbm, wuv_hbm, wo_hbm, kc_hbm, vc_hbm,
            bq_hbm, bo_hbm, g_hbm, out_ref,
            x_s, g_s, c_s, wq_s, wuk_s, wuv_s, wo_s, bq_s, bo_s, k_s, v_s,
            q_s, qa_s, qat_s, cc_s, qb_s, qbt_s, ob_s, oa_s, sems, sem_x):

    def rows_copies(src, dst, nrows, sem, pieces):
        r = nrows // pieces
        return [pltpu.make_async_copy(src.at[pl.ds(i * r, r)], dst.at[pl.ds(i * r, r)], sem)
                for i in range(pieces)]

    def stage_copies(s, b=None):
        sem = sems.at[s % NSEM] if isinstance(s, int) else sems.at[lax.rem(s, NSEM)]
        raise NotImplementedError

    def start_all(copies):
        for i, c in enumerate(copies):
            c.start(priority=i % 2)

    def c_copies(b, sem):
        return rows_copies(ckv_hbm.at[b], c_s.at[b], SK, sem, PIECES)

    def c_wait(b, sem):
        pltpu.make_async_copy(ckv_hbm.at[b], c_s.at[b], sem).wait()

    def kv_copies(b, sem):
        cs = []
        per = PIECES // (2 * HKV) if PIECES >= 2 * HKV else 1
        r = WIN // per
        for h in range(HKV):
            for src, dst in ((kc_hbm, k_s), (vc_hbm, v_s)):
                for i in range(per):
                    cs.append(pltpu.make_async_copy(
                        src.at[b, h, pl.ds(SK - WIN + i * r, r)], dst.at[b, h, pl.ds(i * r, r)], sem))
        return cs

    def kv_wait(b, sem):
        pltpu.make_async_copy(kc_hbm.at[b, :, pl.ds(SK - WIN, WIN)], k_s.at[b], sem).wait()
        pltpu.make_async_copy(vc_hbm.at[b, :, pl.ds(SK - WIN, WIN)], v_s.at[b], sem).wait()

    weights = {0: (wq_hbm, wq_s), 1: (wuk_hbm, wuk_s), 10: (wuv_hbm, wuv_s), 11: (wo_hbm, wo_s),
               12: (bq_hbm, bq_s), 21: (bo_hbm, bo_s)}

    def sem_of(s):
        return sems.at[s % NSEM]

    def start_stage(s):
        if s > 21:
            return
        if s in weights:
            src, dst = weights[s]
            start_all(rows_copies(src, dst, src.shape[0], sem_of(s), PIECES))
        elif s < 10:
            start_all(c_copies(s - 2, sem_of(s)))
        else:
            start_all(kv_copies(s - 13, sem_of(s)))

    def wait_stage(s):
        if s in weights:
            src, dst = weights[s]
            pltpu.make_async_copy(src, dst, sem_of(s)).wait()
        elif s < 10:
            c_wait(s - 2, sem_of(s))
        else:
            kv_wait(s - 13, sem_of(s))

    def advance(s):
        wait_stage(s)
        start_stage(s + LOOKAHEAD)

    cx = pltpu.make_async_copy(x_hbm, x_s, sem_x.at[0])
    cg = pltpu.make_async_copy(g_hbm, g_s, sem_x.at[1])
    for s in range(LOOKAHEAD):
        start_stage(s)
    cx.start()
    cg.start()
    cx.wait()
    cg.wait()
    x = x_s[...]

    advance(0)
    wq_u = wq_s.bitcast(U32)

    def q_body(j, _):
        lo, hi = _unpack_pair(wq_u, j)
        q0 = jnp.dot(x, lo, preferred_element_type=F32)
        q1 = jnp.dot(x, hi, preferred_element_type=F32)
        q_s[pl.ds(j * 16, 16), :] = jnp.concatenate([q0, q1], axis=0)
        return 0
    for j in range(NH // 2):
        q_body(j, 0)

    advance(1)
    wuk_u = wuk_s.bitcast(U32)
    sc_a = (HD ** -0.5) * LOG2E

    def qa_body(j, _):
        lo, hi = _unpack_pair(wuk_u, j)
        q = q_s[pl.ds(j * 16, 16), :].astype(BF16)
        a0 = lax.dot_general(q[0:8], lo, NT, preferred_element_type=F32)
        a1 = lax.dot_general(q[8:16], hi, NT, preferred_element_type=F32)
        a = jnp.concatenate([a0, a1], axis=0) * sc_a
        for t in range(DC // HD):
            qa_s[t, pl.ds(j * 16, 16), :] = a[:, t * HD:(t + 1) * HD]
        return 0
    for j in range(NH // 2):
        qa_body(j, 0)
    for b in range(NB):
        qat_s[b] = jnp.concatenate([qa_s[t, pl.ds(b, NH, stride=NB), :] for t in range(DC // HD)],
                                   axis=1).astype(BF16)

    def a_body(b, _):
        sem = sems.at[lax.rem(b + 2, NSEM)]
        c_wait(b, sem)

        @pl.when(b + LOOKAHEAD < NB)
        def _():
            start_all(c_copies(b + LOOKAHEAD, sems.at[lax.rem(b + 2 + LOOKAHEAD, NSEM)]))
        for t in range(LOOKAHEAD):
            @pl.when(b == NB - LOOKAHEAD + t)
            def _():
                start_stage(10 + t)

        c = c_s[b]
        s = lax.dot_general(qat_s[b], c, NT, preferred_element_type=F32)
        m = jnp.max(s, axis=1, keepdims=True)
        p = jnp.exp2(s - m)
        l = jnp.sum(p, axis=1, keepdims=True)
        ctx = jnp.dot(p.astype(BF16), c, preferred_element_type=F32)
        ctx = ctx / l
        for t in range(DC // HD):
            cc_s[t, pl.ds(pl.multiple_of(b * NH, NH), NH), :] = ctx[:, t * HD:(t + 1) * HD]
        return 0
    lax.fori_loop(0, NB, a_body, 0)

    advance(10)
    wuv_u = wuv_s.bitcast(U32)

    def uv_body(j, _):
        lo, hi = _unpack_pair(wuv_u, j)
        c0 = jnp.concatenate([cc_s[t, pl.ds(2 * j, NB, stride=NH), :] for t in range(DC // HD)],
                             axis=1).astype(BF16)
        c1 = jnp.concatenate([cc_s[t, pl.ds(2 * j + 1, NB, stride=NH), :] for t in range(DC // HD)],
                             axis=1).astype(BF16)
        o0 = jnp.dot(c0, lo, preferred_element_type=F32)
        o1 = jnp.dot(c1, hi, preferred_element_type=F32)
        oa_s[:, pl.ds(j * 256, 256)] = jnp.concatenate([o0, o1], axis=1)
        return 0
    for j in range(NH // 2):
        uv_body(j, 0)

    advance(11)
    out_a = jnp.dot(oa_s[...].astype(BF16), wo_s[...], preferred_element_type=F32)

    advance(12)
    sc_b = (HD ** -0.5) * LOG2E
    qb = jnp.dot(x, bq_s[...], preferred_element_type=F32)
    qb = qb.astype(BF16).astype(F32) * sc_b
    for h in range(NH):
        qb_s[h * NB:(h + 1) * NB, :] = qb[:, h * HD:(h + 1) * HD]
    for b in range(NB):
        qbt_s[b] = qb_s[pl.ds(b, NH, stride=NB), :]

    row = lax.broadcasted_iota(jnp.int32, (8, HD), 0)
    row_w = lax.broadcasted_iota(jnp.int32, (8, WIN), 0)

    def b_body(b, _):
        kv_wait(b, sems.at[lax.rem(b + 13, NSEM)])

        @pl.when(b + LOOKAHEAD < NB)
        def _():
            start_all(kv_copies(b + LOOKAHEAD, sems.at[lax.rem(b + 13 + LOOKAHEAD, NSEM)]))

        @pl.when(b == NB - LOOKAHEAD)
        def _():
            start_stage(21)

        for i in range(HKV // 2):
            q8 = qbt_s[b, 8 * i:8 * (i + 1), :]
            q0 = jnp.where(row < 4, q8, 0.0).astype(BF16)
            q1 = jnp.where(row >= 4, q8, 0.0).astype(BF16)
            s = (lax.dot_general(q0, k_s[b, 2 * i], NT, preferred_element_type=F32)
                 + lax.dot_general(q1, k_s[b, 2 * i + 1], NT, preferred_element_type=F32))
            m = jnp.max(s, axis=1, keepdims=True)
            p = jnp.exp2(s - m)
            l = jnp.sum(p, axis=1, keepdims=True)
            p0 = jnp.where(row_w < 4, p, 0.0).astype(BF16)
            p1 = jnp.where(row_w >= 4, p, 0.0).astype(BF16)
            o = (jnp.dot(p0, v_s[b, 2 * i], preferred_element_type=F32)
                 + jnp.dot(p1, v_s[b, 2 * i + 1], preferred_element_type=F32))
            ob_s[pl.ds(pl.multiple_of(b * NH + 8 * i, 8), 8), :] = o / l
        return 0
    lax.fori_loop(0, NB, b_body, 0)

    ob = jnp.concatenate([ob_s[pl.ds(h, NB, stride=NH), :] for h in range(NH)], axis=1).astype(BF16)
    gate = jnp.sum(x.astype(F32) * g_s[...].astype(F32).reshape(1, DM), axis=1, keepdims=True)
    g = 1.0 / (1.0 + jnp.exp(-gate))
    wait_stage(21)
    out_b = jnp.dot(ob, bo_s[...], preferred_element_type=F32)
    out_ref[...] = (g * out_a + (1.0 - g) * out_b).astype(out_ref.dtype)


@jax.jit
def pallas_gated_mix__compressed_kv_cla__sliding_block_cached__decode_kernel(
    A_x, A_c_kv, A_w_q, A_w_uk, A_w_uv, A_w_o, B_x, B_k_cache, B_v_cache, B_wq, B_wo, gate_w,
):
    del B_x
    any_spec = pl.BlockSpec(memory_space=pl.ANY)
    return pl.pallas_call(
        _kernel,
        out_shape=jax.ShapeDtypeStruct((NB, DM), A_x.dtype),
        in_specs=[any_spec] * 11,
        out_specs=pl.BlockSpec(memory_space=pltpu.VMEM),
        scratch_shapes=[
            pltpu.VMEM((NB, DM), BF16),
            pltpu.VMEM((DM,), BF16),
            pltpu.VMEM((NB, SK, DC), BF16),
            pltpu.VMEM((DM * NH, HD), BF16),
            pltpu.VMEM((DC * NH, HD), BF16),
            pltpu.VMEM((DC * NH, HD), BF16),
            pltpu.VMEM((NH * HD, DM), BF16),
            pltpu.VMEM((DM, NH * HD), BF16),
            pltpu.VMEM((NH * HD, DM), BF16),
            pltpu.VMEM((NB, HKV, WIN, HD), BF16),
            pltpu.VMEM((NB, HKV, WIN, HD), BF16),
            pltpu.VMEM((NH * NB, HD), F32),
            pltpu.VMEM((DC // HD, NH * NB, HD), F32),
            pltpu.VMEM((NB, NH, DC), BF16),
            pltpu.VMEM((DC // HD, NB * NH, HD), F32),
            pltpu.VMEM((NH * NB, HD), F32),
            pltpu.VMEM((NB, NH, HD), F32),
            pltpu.VMEM((NB * NH, HD), F32),
            pltpu.VMEM((NB, NH * HD), F32),
            pltpu.SemaphoreType.DMA((NSEM,)),
            pltpu.SemaphoreType.DMA((2,)),
        ],
        compiler_params=pltpu.CompilerParams(vmem_limit_bytes=120 * 1024 * 1024),
    )(
        A_x.reshape(NB, DM),
        A_c_kv,
        A_w_q.reshape(DM * NH, HD),
        A_w_uk.reshape(DC * NH, HD),
        A_w_uv.reshape(DC * NH, HD),
        A_w_o.reshape(NH * HD, DM),
        B_k_cache,
        B_v_cache,
        B_wq,
        B_wo,
        gate_w,
    ).reshape(NB, 1, DM)
```

```python
import math

import jax
import jax.numpy as jnp
from jax import lax
import jax.experimental.pallas as pl
import jax.experimental.pallas.tpu as pltpu

F32 = jnp.float32
BF16 = jnp.bfloat16
U32 = jnp.uint32
NT = (((1,), (1,)), ((), ()))
LOG2E = math.log2(math.e)

NB = 8
SK = 4096
DC = 512
NH = 32
HD = 128
DM = 512
HKV = 8
WIN = 1024

PIECE_BYTES = 32 * 1024
AHEAD = 4
NSEM = 4
TAILG = 16
TAILR = NH * HD // 2 // TAILG

S_WQ, S_WUK, S_C0, S_WUV, S_BQ, S_KV0, S_WO, S_BO = 0, 1, 2, 10, 11, 12, 20, 21


def _unpack_pair(w_u32, j):
    u = w_u32[pl.ds(j, 512, stride=16), :]
    lo = pltpu.bitcast(u << 16, F32).astype(BF16)
    hi = pltpu.bitcast(u & jnp.uint32(0xFFFF0000), F32).astype(BF16)
    return lo, hi


def _kernel(x_hbm, ckv_hbm, wq_hbm, wuk_hbm, wuv_hbm, wo_hbm, kc_hbm, vc_hbm,
            bq_hbm, bo_hbm, g_hbm, out_ref,
            x_s, g_s, c_s, wq_s, wuk_s, wuv_s, wo_s, bq_s, bo_s, k_s, v_s,
            q_s, qa_s, qat_s, s_s, cc_s, qb_s, qbt_s, ob_s, oa_s, sems, sem_x, tail_sems):

    def issue_rows(src, dst, sem, base, count):
        r = max(PIECE_BYTES // (2 * src.shape[1]), 16)
        half = src.shape[0] // 2
        for i in range(count // r):
            o = base + i * r
            pltpu.make_async_copy(src.at[pl.ds(o, r)], dst.at[pl.ds(o, r)], sem).start(priority=0)
            pltpu.make_async_copy(src.at[pl.ds(half + o, r)], dst.at[pl.ds(half + o, r)],
                                  sem).start(priority=1)

    def issue_rows_quarter(src, dst, sem, k):
        q = src.shape[0] // 8
        issue_rows(src, dst, sem, k * q, q)

    def issue_kv_quarter(b, sem, k):
        r = PIECE_BYTES // (2 * HD)
        for h in range(2 * k, 2 * k + 2):
            for i in range(WIN // r):
                o = i * r
                pltpu.make_async_copy(kc_hbm.at[b, h, pl.ds(SK - WIN + o, r)],
                                      k_s.at[b, h, pl.ds(o, r)], sem).start(priority=0)
                pltpu.make_async_copy(vc_hbm.at[b, h, pl.ds(SK - WIN + o, r)],
                                      v_s.at[b, h, pl.ds(o, r)], sem).start(priority=1)

    def c_wait(b, sem):
        pltpu.make_async_copy(ckv_hbm.at[b], c_s.at[b], sem).wait()

    def kv_wait(b, sem):
        pltpu.make_async_copy(kc_hbm.at[b, :, pl.ds(SK - WIN, WIN)], k_s.at[b], sem).wait()
        pltpu.make_async_copy(vc_hbm.at[b, :, pl.ds(SK - WIN, WIN)], v_s.at[b], sem).wait()

    weights = {S_WQ: (wq_hbm, wq_s), S_WUK: (wuk_hbm, wuk_s), S_WUV: (wuv_hbm, wuv_s),
               S_WO: (wo_hbm, wo_s), S_BQ: (bq_hbm, bq_s)}

    def sem_of(s):
        return sems.at[s % NSEM]

    def sem_dyn(s):
        return sems.at[lax.rem(s, NSEM)]

    def issue_quarter(s, k):
        if s > S_BO:
            return
        if s == S_BO:
            per = TAILG // 4
            for i in range(k * per, (k + 1) * per):
                issue_rows(bo_hbm, bo_s, tail_sems.at[i], i * TAILR, TAILR)
        elif s in weights:
            issue_rows_quarter(*weights[s], sem_of(s), k)
        elif s < S_WUV:
            issue_rows_quarter(ckv_hbm.at[s - S_C0], c_s.at[s - S_C0], sem_of(s), k)
        else:
            issue_kv_quarter(s - S_KV0, sem_of(s), k)

    def wait_stage(s):
        src, dst = weights[s]
        pltpu.make_async_copy(src, dst, sem_of(s)).wait()

    def issue_after_block(s, k):
        g = 4 + AHEAD + k
        issue_quarter(s + g // 4, g % 4)

    def issue_after_block_loop(s0, n, b, k, issue_same):
        g = 4 + AHEAD + k
        d, kk = g // 4, g % 4

        @pl.when(b + d < n)
        def _():
            issue_same(b + d, sem_dyn(s0 + b + d), kk)
        for t in range(d):
            @pl.when(b == n - d + t)
            def _():
                issue_quarter(s0 + n + t, kk)

    cx = pltpu.make_async_copy(x_hbm, x_s, sem_x.at[0])
    cg = pltpu.make_async_copy(g_hbm, g_s, sem_x.at[1])
    issue_quarter(S_WQ, 0)
    for k in range(1, 4):
        issue_quarter(S_WQ, k)
    for g in range(AHEAD):
        issue_quarter(S_WUK + g // 4, g % 4)
    cx.start()
    cg.start()
    cx.wait()
    cg.wait()
    x = x_s[...]

    wait_stage(S_WQ)
    wq_u = wq_s.bitcast(U32)
    for k in range(4):
        issue_after_block(S_WQ, k)
        for j in range(4 * k, 4 * k + 4):
            lo, hi = _unpack_pair(wq_u, j)
            q0 = jnp.dot(x, lo, preferred_element_type=F32)
            q1 = jnp.dot(x, hi, preferred_element_type=F32)
            q_s[pl.ds(j * 16, 16), :] = jnp.concatenate([q0, q1], axis=0)

    wait_stage(S_WUK)
    wuk_u = wuk_s.bitcast(U32)
    sc_a = (HD ** -0.5) * LOG2E
    for k in range(4):
        issue_after_block(S_WUK, k)
        for j in range(4 * k, 4 * k + 4):
            lo, hi = _unpack_pair(wuk_u, j)
            q = q_s[pl.ds(j * 16, 16), :].astype(BF16)
            a0 = lax.dot_general(q[0:8], lo, NT, preferred_element_type=F32)
            a1 = lax.dot_general(q[8:16], hi, NT, preferred_element_type=F32)
            a = jnp.concatenate([a0, a1], axis=0) * sc_a
            for t in range(DC // HD):
                qa_s[t, pl.ds(j * 16, 16), :] = a[:, t * HD:(t + 1) * HD]
        if k == 3:
            for b in range(NB):
                qat_s[b] = jnp.concatenate(
                    [qa_s[t, pl.ds(b, NH, stride=NB), :] for t in range(DC // HD)], axis=1).astype(BF16)

    def c_issue(b, sem, k):
        issue_rows_quarter(ckv_hbm.at[b], c_s.at[b], sem, k)

    HK = SK // 2

    def a_body(b, carry):
        c_wait(b, sem_dyn(S_C0 + b))
        nxt = lambda k: issue_after_block_loop(S_C0, NB, b, k, c_issue)
        nxt(0)
        qa = qat_s[b]
        s0 = lax.dot_general(qa, c_s[b, 0:HK, :], NT, preferred_element_type=F32)
        m0 = jnp.max(s0, axis=1, keepdims=True)
        s_s[:, 0:HK] = s0
        nxt(1)
        s1 = lax.dot_general(qa, c_s[b, HK:SK, :], NT, preferred_element_type=F32)
        m = jnp.maximum(m0, jnp.max(s1, axis=1, keepdims=True))
        nxt(2)
        p1 = jnp.exp2(s1 - m)
        l = jnp.sum(p1, axis=1, keepdims=True)
        ctx = jnp.dot(p1.astype(BF16), c_s[b, HK:SK, :], preferred_element_type=F32)
        nxt(3)
        p0 = jnp.exp2(s_s[:, 0:HK] - m)
        l = l + jnp.sum(p0, axis=1, keepdims=True)
        ctx = ctx + jnp.dot(p0.astype(BF16), c_s[b, 0:HK, :], preferred_element_type=F32)
        ctx = ctx / l
        for t in range(DC // HD):
            cc_s[t, pl.ds(pl.multiple_of(b * NH, NH), NH), :] = ctx[:, t * HD:(t + 1) * HD]
        return carry
    lax.fori_loop(0, NB, a_body, 0)

    wait_stage(S_WUV)
    wuv_u = wuv_s.bitcast(U32)
    for k in range(4):
        issue_after_block(S_WUV, k)
        for j in range(4 * k, 4 * k + 4):
            lo, hi = _unpack_pair(wuv_u, j)
            c0 = jnp.concatenate([cc_s[t, pl.ds(2 * j, NB, stride=NH), :] for t in range(DC // HD)],
                                 axis=1).astype(BF16)
            c1 = jnp.concatenate([cc_s[t, pl.ds(2 * j + 1, NB, stride=NH), :] for t in range(DC // HD)],
                                 axis=1).astype(BF16)
            o0 = jnp.dot(c0, lo, preferred_element_type=F32)
            o1 = jnp.dot(c1, hi, preferred_element_type=F32)
            oa_s[:, pl.ds(j * 256, 256)] = jnp.concatenate([o0, o1], axis=1)

    wait_stage(S_BQ)
    sc_b = (HD ** -0.5) * LOG2E
    KC = NH * HD // 4
    for k in range(4):
        issue_after_block(S_BQ, k)
        qb = jnp.dot(x, bq_s[:, k * KC:(k + 1) * KC], preferred_element_type=F32)
        qb = qb.astype(BF16).astype(F32) * sc_b
        for hh in range(KC // HD):
            h = k * (KC // HD) + hh
            qb_s[h * NB:(h + 1) * NB, :] = qb[:, hh * HD:(hh + 1) * HD]
        if k == 3:
            for b in range(NB):
                qbt_s[b] = qb_s[pl.ds(b, NH, stride=NB), :]

    row = lax.broadcasted_iota(jnp.int32, (8, HD), 0)
    row_w = lax.broadcasted_iota(jnp.int32, (8, WIN), 0)

    def b_body(b, carry):
        kv_wait(b, sem_dyn(S_KV0 + b))
        for i in range(HKV // 2):
            issue_after_block_loop(S_KV0, NB, b, i, issue_kv_quarter)
            q8 = qbt_s[b, 8 * i:8 * (i + 1), :]
            q0 = jnp.where(row < 4, q8, 0.0).astype(BF16)
            q1 = jnp.where(row >= 4, q8, 0.0).astype(BF16)
            s = (lax.dot_general(q0, k_s[b, 2 * i], NT, preferred_element_type=F32)
                 + lax.dot_general(q1, k_s[b, 2 * i + 1], NT, preferred_element_type=F32))
            m = jnp.max(s, axis=1, keepdims=True)
            p = jnp.exp2(s - m)
            l = jnp.sum(p, axis=1, keepdims=True)
            p0 = jnp.where(row_w < 4, p, 0.0).astype(BF16)
            p1 = jnp.where(row_w >= 4, p, 0.0).astype(BF16)
            o = (jnp.dot(p0, v_s[b, 2 * i], preferred_element_type=F32)
                 + jnp.dot(p1, v_s[b, 2 * i + 1], preferred_element_type=F32))
            ob_s[pl.ds(pl.multiple_of(b * NH + 8 * i, 8), 8), :] = o / l
        return carry
    lax.fori_loop(0, NB, b_body, 0)

    ob = jnp.concatenate([ob_s[pl.ds(h, NB, stride=NH), :] for h in range(NH)], axis=1).astype(BF16)
    gate = jnp.sum(x.astype(F32) * g_s[...].astype(F32).reshape(1, DM), axis=1, keepdims=True)
    g = 1.0 / (1.0 + jnp.exp(-gate))
    wait_stage(S_WO)
    out_a = jnp.zeros((NB, DM), F32)
    for k in range(4):
        issue_after_block(S_WO, k)
        out_a += jnp.dot(oa_s[:, k * KC:(k + 1) * KC].astype(BF16), wo_s[k * KC:(k + 1) * KC, :],
                         preferred_element_type=F32)

    out_b = jnp.zeros((NB, DM), F32)
    for i in range(TAILG):
        lo0, hi0 = i * TAILR, NH * HD // 2 + i * TAILR
        pltpu.make_async_copy(bo_hbm.at[pl.ds(0, 2 * TAILR)], bo_s.at[pl.ds(0, 2 * TAILR)],
                              tail_sems.at[i]).wait()
        out_b += jnp.dot(ob[:, lo0:lo0 + TAILR], bo_s[lo0:lo0 + TAILR, :], preferred_element_type=F32)
        out_b += jnp.dot(ob[:, hi0:hi0 + TAILR], bo_s[hi0:hi0 + TAILR, :], preferred_element_type=F32)
    out_ref[...] = (g * out_a + (1.0 - g) * out_b).astype(out_ref.dtype)


@jax.jit
def pallas_gated_mix__compressed_kv_cla__sliding_block_cached__decode_kernel(
    A_x, A_c_kv, A_w_q, A_w_uk, A_w_uv, A_w_o, B_x, B_k_cache, B_v_cache, B_wq, B_wo, gate_w,
):
    del B_x
    any_spec = pl.BlockSpec(memory_space=pl.ANY)
    return pl.pallas_call(
        _kernel,
        out_shape=jax.ShapeDtypeStruct((NB, DM), A_x.dtype),
        in_specs=[any_spec] * 11,
        out_specs=pl.BlockSpec(memory_space=pltpu.VMEM),
        scratch_shapes=[
            pltpu.VMEM((NB, DM), BF16),
            pltpu.VMEM((DM,), BF16),
            pltpu.VMEM((NB, SK, DC), BF16),
            pltpu.VMEM((DM * NH, HD), BF16),
            pltpu.VMEM((DC * NH, HD), BF16),
            pltpu.VMEM((DC * NH, HD), BF16),
            pltpu.VMEM((NH * HD, DM), BF16),
            pltpu.VMEM((DM, NH * HD), BF16),
            pltpu.VMEM((NH * HD, DM), BF16),
            pltpu.VMEM((NB, HKV, WIN, HD), BF16),
            pltpu.VMEM((NB, HKV, WIN, HD), BF16),
            pltpu.VMEM((NH * NB, HD), F32),
            pltpu.VMEM((DC // HD, NH * NB, HD), F32),
            pltpu.VMEM((NB, NH, DC), BF16),
            pltpu.VMEM((NH, SK // 2), F32),
            pltpu.VMEM((DC // HD, NB * NH, HD), F32),
            pltpu.VMEM((NH * NB, HD), F32),
            pltpu.VMEM((NB, NH, HD), F32),
            pltpu.VMEM((NB * NH, HD), F32),
            pltpu.VMEM((NB, NH * HD), F32),
            pltpu.SemaphoreType.DMA((NSEM,)),
            pltpu.SemaphoreType.DMA((2,)),
            pltpu.SemaphoreType.DMA((TAILG,)),
        ],
        compiler_params=pltpu.CompilerParams(vmem_limit_bytes=120 * 1024 * 1024,
                                             disable_semaphore_checks=True),
    )(
        A_x.reshape(NB, DM),
        A_c_kv,
        A_w_q.reshape(DM * NH, HD),
        A_w_uk.reshape(DC * NH, HD),
        A_w_uv.reshape(DC * NH, HD),
        A_w_o.reshape(NH * HD, DM),
        B_k_cache,
        B_v_cache,
        B_wq,
        B_wo,
        gate_w,
    ).reshape(NB, 1, DM)
```

```python
import math

import jax
import jax.numpy as jnp
from jax import lax
import jax.experimental.pallas as pl
import jax.experimental.pallas.tpu as pltpu

F32 = jnp.float32
BF16 = jnp.bfloat16
U32 = jnp.uint32
NT = (((1,), (1,)), ((), ()))
LOG2E = math.log2(math.e)

NB = 8
SK = 4096
DC = 512
NH = 32
HD = 128
DM = 512
HKV = 8
WIN = 1024

P256 = (48,)
P1K = (48,)
PKV = (44,)
PTAIL = (48,)
PWIDE = (48,)
AHEAD = 4
NSEM = 4
TAILG = 16
TAILR = NH * HD // 2 // TAILG

S_WQ, S_WUK, S_C0, S_WUV, S_BQ, S_KV0, S_WO, S_BO = 0, 1, 2, 10, 11, 12, 20, 21


def _plan(base, count, sizes_kib, row_bytes):
    out, o, i = [], base, 0
    while o < base + count:
        n = min(sizes_kib[i % len(sizes_kib)] * 1024 // row_bytes, base + count - o)
        out.append((o, n))
        o += n
        i += 1
    return out


def _unpack_pair(w_u32, j):
    u = w_u32[pl.ds(j, 512, stride=16), :]
    lo = pltpu.bitcast(u << 16, F32).astype(BF16)
    hi = pltpu.bitcast(u & jnp.uint32(0xFFFF0000), F32).astype(BF16)
    return lo, hi


def _kernel(x_hbm, ckv_hbm, wq_hbm, wuk_hbm, wuv_hbm, wo_hbm, kc_hbm, vc_hbm,
            bq_hbm, bo_hbm, g_hbm, out_ref,
            x_s, g_s, c_s, wq_s, wuk_s, wuv_s, wo_s, bq_s, bo_s, k_s, v_s,
            q_s, qa_s, qat_s, s_s, cc_s, qb_s, qbt_s, ob_s, oa_s, sems, sem_x, tail_sems):

    def issue_rows(src, dst, sem, base, count):
        half = src.shape[0] // 2
        row_bytes = 2 * src.shape[1]
        if row_bytes == 8192:
            for o in range(base, base + count, 8):
                for c0, w in _plan(0, src.shape[1], PWIDE, 16):
                    for r0, prio in ((o, 0), (half + o, 1)):
                        pltpu.make_async_copy(src.at[pl.ds(r0, 8), pl.ds(c0, w)],
                                              dst.at[pl.ds(r0, 8), pl.ds(c0, w)], sem).start(priority=prio)
            return
        pb = PTAIL if dst is bo_s else (P256 if row_bytes == 256 else P1K)
        for o, n in _plan(base, count, pb, row_bytes):
            for r0, prio in ((o, 0), (half + o, 1)):
                pltpu.make_async_copy(src.at[pl.ds(r0, n)], dst.at[pl.ds(r0, n)], sem).start(priority=prio)

    def issue_rows_quarter(src, dst, sem, k):
        q = src.shape[0] // 8
        issue_rows(src, dst, sem, k * q, q)

    def issue_kv_quarter(b, sem, k):
        for h in range(2 * k, 2 * k + 2):
            for o, n in _plan(0, WIN, PKV, 2 * HD):
                pltpu.make_async_copy(kc_hbm.at[b, h, pl.ds(SK - WIN + o, n)],
                                      k_s.at[b, h, pl.ds(o, n)], sem).start(priority=0)
                pltpu.make_async_copy(vc_hbm.at[b, h, pl.ds(SK - WIN + o, n)],
                                      v_s.at[b, h, pl.ds(o, n)], sem).start(priority=1)

    def c_wait(b, sem):
        pltpu.make_async_copy(ckv_hbm.at[b], c_s.at[b], sem).wait()

    def kv_wait(b, sem):
        pltpu.make_async_copy(kc_hbm.at[b, :, pl.ds(SK - WIN, WIN)], k_s.at[b], sem).wait()
        pltpu.make_async_copy(vc_hbm.at[b, :, pl.ds(SK - WIN, WIN)], v_s.at[b], sem).wait()

    weights = {S_WQ: (wq_hbm, wq_s), S_WUK: (wuk_hbm, wuk_s), S_WUV: (wuv_hbm, wuv_s),
               S_WO: (wo_hbm, wo_s), S_BQ: (bq_hbm, bq_s)}

    def sem_of(s):
        return sems.at[s % NSEM]

    def sem_dyn(s):
        return sems.at[lax.rem(s, NSEM)]

    def issue_quarter(s, k):
        if s > S_BO:
            return
        if s == S_BO:
            per = TAILG // 4
            for i in range(k * per, (k + 1) * per):
                issue_rows(bo_hbm, bo_s, tail_sems.at[i], i * TAILR, TAILR)
        elif s in weights:
            issue_rows_quarter(*weights[s], sem_of(s), k)
        elif s < S_WUV:
            issue_rows_quarter(ckv_hbm.at[s - S_C0], c_s.at[s - S_C0], sem_of(s), k)
        else:
            issue_kv_quarter(s - S_KV0, sem_of(s), k)

    def wait_stage(s):
        src, dst = weights[s]
        pltpu.make_async_copy(src, dst, sem_of(s)).wait()

    def issue_after_block(s, k):
        g = 4 + AHEAD + k
        issue_quarter(s + g // 4, g % 4)

    def issue_after_block_loop(s0, n, b, k, issue_same):
        g = 4 + AHEAD + k
        d, kk = g // 4, g % 4

        @pl.when(b + d < n)
        def _():
            issue_same(b + d, sem_dyn(s0 + b + d), kk)
        for t in range(d):
            @pl.when(b == n - d + t)
            def _():
                issue_quarter(s0 + n + t, kk)

    cx = pltpu.make_async_copy(x_hbm, x_s, sem_x.at[0])
    cg = pltpu.make_async_copy(g_hbm, g_s, sem_x.at[1])
    issue_quarter(S_WQ, 0)
    for k in range(1, 4):
        issue_quarter(S_WQ, k)
    for g in range(AHEAD):
        issue_quarter(S_WUK + g // 4, g % 4)
    cx.start()
    cg.start()
    cx.wait()
    cg.wait()
    x = x_s[...]

    wait_stage(S_WQ)
    wq_u = wq_s.bitcast(U32)
    for k in range(4):
        issue_after_block(S_WQ, k)
        for j in range(4 * k, 4 * k + 4):
            lo, hi = _unpack_pair(wq_u, j)
            q0 = jnp.dot(x, lo, preferred_element_type=F32)
            q1 = jnp.dot(x, hi, preferred_element_type=F32)
            q_s[pl.ds(j * 16, 16), :] = jnp.concatenate([q0, q1], axis=0)

    wait_stage(S_WUK)
    wuk_u = wuk_s.bitcast(U32)
    sc_a = (HD ** -0.5) * LOG2E
    for k in range(4):
        issue_after_block(S_WUK, k)
        for j in range(4 * k, 4 * k + 4):
            lo, hi = _unpack_pair(wuk_u, j)
            q = q_s[pl.ds(j * 16, 16), :].astype(BF16)
            a0 = lax.dot_general(q[0:8], lo, NT, preferred_element_type=F32)
            a1 = lax.dot_general(q[8:16], hi, NT, preferred_element_type=F32)
            a = jnp.concatenate([a0, a1], axis=0) * sc_a
            for t in range(DC // HD):
                qa_s[t, pl.ds(j * 16, 16), :] = a[:, t * HD:(t + 1) * HD]
        if k == 3:
            for b in range(NB):
                qat_s[b] = jnp.concatenate(
                    [qa_s[t, pl.ds(b, NH, stride=NB), :] for t in range(DC // HD)], axis=1).astype(BF16)

    def c_issue(b, sem, k):
        issue_rows_quarter(ckv_hbm.at[b], c_s.at[b], sem, k)

    HK = SK // 2

    def a_body(b, carry):
        c_wait(b, sem_dyn(S_C0 + b))
        nxt = lambda k: issue_after_block_loop(S_C0, NB, b, k, c_issue)
        nxt(0)
        qa = qat_s[b]
        s0 = lax.dot_general(qa, c_s[b, 0:HK, :], NT, preferred_element_type=F32)
        m0 = jnp.max(s0, axis=1, keepdims=True)
        s_s[:, 0:HK] = s0
        nxt(1)
        s1 = lax.dot_general(qa, c_s[b, HK:SK, :], NT, preferred_element_type=F32)
        m = jnp.maximum(m0, jnp.max(s1, axis=1, keepdims=True))
        nxt(2)
        p1 = jnp.exp2(s1 - m)
        l = jnp.sum(p1, axis=1, keepdims=True)
        ctx = jnp.dot(p1.astype(BF16), c_s[b, HK:SK, :], preferred_element_type=F32)
        nxt(3)
        p0 = jnp.exp2(s_s[:, 0:HK] - m)
        l = l + jnp.sum(p0, axis=1, keepdims=True)
        ctx = ctx + jnp.dot(p0.astype(BF16), c_s[b, 0:HK, :], preferred_element_type=F32)
        ctx = ctx / l
        for t in range(DC // HD):
            cc_s[t, pl.ds(pl.multiple_of(b * NH, NH), NH), :] = ctx[:, t * HD:(t + 1) * HD]
        return carry
    lax.fori_loop(0, NB, a_body, 0)

    wait_stage(S_WUV)
    wuv_u = wuv_s.bitcast(U32)
    for k in range(4):
        issue_after_block(S_WUV, k)
        for j in range(4 * k, 4 * k + 4):
            lo, hi = _unpack_pair(wuv_u, j)
            c0 = jnp.concatenate([cc_s[t, pl.ds(2 * j, NB, stride=NH), :] for t in range(DC // HD)],
                                 axis=1).astype(BF16)
            c1 = jnp.concatenate([cc_s[t, pl.ds(2 * j + 1, NB, stride=NH), :] for t in range(DC // HD)],
                                 axis=1).astype(BF16)
            o0 = jnp.dot(c0, lo, preferred_element_type=F32)
            o1 = jnp.dot(c1, hi, preferred_element_type=F32)
            oa_s[:, pl.ds(j * 256, 256)] = jnp.concatenate([o0, o1], axis=1)

    wait_stage(S_BQ)
    sc_b = (HD ** -0.5) * LOG2E
    KC = NH * HD // 4
    for k in range(4):
        issue_after_block(S_BQ, k)
        qb = jnp.dot(x, bq_s[:, k * KC:(k + 1) * KC], preferred_element_type=F32)
        qb = qb.astype(BF16).astype(F32) * sc_b
        for hh in range(KC // HD):
            h = k * (KC // HD) + hh
            qb_s[h * NB:(h + 1) * NB, :] = qb[:, hh * HD:(hh + 1) * HD]
        if k == 3:
            for b in range(NB):
                qbt_s[b] = qb_s[pl.ds(b, NH, stride=NB), :]

    row = lax.broadcasted_iota(jnp.int32, (8, HD), 0)
    row_w = lax.broadcasted_iota(jnp.int32, (8, WIN), 0)

    def b_body(b, carry):
        kv_wait(b, sem_dyn(S_KV0 + b))
        for i in range(HKV // 2):
            issue_after_block_loop(S_KV0, NB, b, i, issue_kv_quarter)
            q8 = qbt_s[b, 8 * i:8 * (i + 1), :]
            q0 = jnp.where(row < 4, q8, 0.0).astype(BF16)
            q1 = jnp.where(row >= 4, q8, 0.0).astype(BF16)
            s = (lax.dot_general(q0, k_s[b, 2 * i], NT, preferred_element_type=F32)
                 + lax.dot_general(q1, k_s[b, 2 * i + 1], NT, preferred_element_type=F32))
            m = jnp.max(s, axis=1, keepdims=True)
            p = jnp.exp2(s - m)
            l = jnp.sum(p, axis=1, keepdims=True)
            p0 = jnp.where(row_w < 4, p, 0.0).astype(BF16)
            p1 = jnp.where(row_w >= 4, p, 0.0).astype(BF16)
            o = (jnp.dot(p0, v_s[b, 2 * i], preferred_element_type=F32)
                 + jnp.dot(p1, v_s[b, 2 * i + 1], preferred_element_type=F32))
            ob_s[pl.ds(pl.multiple_of(b * NH + 8 * i, 8), 8), :] = o / l
        return carry
    lax.fori_loop(0, NB, b_body, 0)

    ob = jnp.concatenate([ob_s[pl.ds(h, NB, stride=NH), :] for h in range(NH)], axis=1).astype(BF16)
    gate = jnp.sum(x.astype(F32) * g_s[...].astype(F32).reshape(1, DM), axis=1, keepdims=True)
    g = jax.nn.sigmoid(gate)
    wait_stage(S_WO)
    out_a = jnp.zeros((NB, DM), F32)
    for k in range(4):
        issue_after_block(S_WO, k)
        out_a += jnp.dot(oa_s[:, k * KC:(k + 1) * KC].astype(BF16), wo_s[k * KC:(k + 1) * KC, :],
                         preferred_element_type=F32)

    out_b = jnp.zeros((NB, DM), F32)
    for i in range(TAILG):
        lo0, hi0 = i * TAILR, NH * HD // 2 + i * TAILR
        for r0 in (lo0, hi0):
            pltpu.make_async_copy(bo_hbm.at[pl.ds(r0, TAILR)], bo_s.at[pl.ds(r0, TAILR)],
                                  tail_sems.at[i]).wait()
        out_b += jnp.dot(ob[:, lo0:lo0 + TAILR], bo_s[lo0:lo0 + TAILR, :], preferred_element_type=F32)
        out_b += jnp.dot(ob[:, hi0:hi0 + TAILR], bo_s[hi0:hi0 + TAILR, :], preferred_element_type=F32)
    out_ref[...] = (g * out_a + (1.0 - g) * out_b).astype(out_ref.dtype)


@jax.jit
def pallas_gated_mix__compressed_kv_cla__sliding_block_cached__decode_kernel(
    A_x, A_c_kv, A_w_q, A_w_uk, A_w_uv, A_w_o, B_x, B_k_cache, B_v_cache, B_wq, B_wo, gate_w,
):
    del B_x
    any_spec = pl.BlockSpec(memory_space=pl.ANY)
    return pl.pallas_call(
        _kernel,
        out_shape=jax.ShapeDtypeStruct((NB, DM), A_x.dtype),
        in_specs=[any_spec] * 11,
        out_specs=pl.BlockSpec(memory_space=pltpu.VMEM),
        scratch_shapes=[
            pltpu.VMEM((NB, DM), BF16),
            pltpu.VMEM((DM,), BF16),
            pltpu.VMEM((NB, SK, DC), BF16),
            pltpu.VMEM((DM * NH, HD), BF16),
            pltpu.VMEM((DC * NH, HD), BF16),
            pltpu.VMEM((DC * NH, HD), BF16),
            pltpu.VMEM((NH * HD, DM), BF16),
            pltpu.VMEM((DM, NH * HD), BF16),
            pltpu.VMEM((NH * HD, DM), BF16),
            pltpu.VMEM((NB, HKV, WIN, HD), BF16),
            pltpu.VMEM((NB, HKV, WIN, HD), BF16),
            pltpu.VMEM((NH * NB, HD), F32),
            pltpu.VMEM((DC // HD, NH * NB, HD), F32),
            pltpu.VMEM((NB, NH, DC), BF16),
            pltpu.VMEM((NH, SK // 2), F32),
            pltpu.VMEM((DC // HD, NB * NH, HD), F32),
            pltpu.VMEM((NH * NB, HD), F32),
            pltpu.VMEM((NB, NH, HD), F32),
            pltpu.VMEM((NB * NH, HD), F32),
            pltpu.VMEM((NB, NH * HD), F32),
            pltpu.SemaphoreType.DMA((NSEM,)),
            pltpu.SemaphoreType.DMA((2,)),
            pltpu.SemaphoreType.DMA((TAILG,)),
        ],
        compiler_params=pltpu.CompilerParams(vmem_limit_bytes=120 * 1024 * 1024,
                                             disable_semaphore_checks=True),
    )(
        A_x.reshape(NB, DM),
        A_c_kv,
        A_w_q.reshape(DM * NH, HD),
        A_w_uk.reshape(DC * NH, HD),
        A_w_uv.reshape(DC * NH, HD),
        A_w_o.reshape(NH * HD, DM),
        B_k_cache,
        B_v_cache,
        B_wq,
        B_wo,
        gate_w,
    ).reshape(NB, 1, DM)
```

```python
import math

import jax
import jax.numpy as jnp
from jax import lax
import jax.experimental.pallas as pl
import jax.experimental.pallas.tpu as pltpu

F32 = jnp.float32
BF16 = jnp.bfloat16
U32 = jnp.uint32
NT = (((1,), (1,)), ((), ()))
LOG2E = math.log2(math.e)

NB = 8
SK = 4096
DC = 512
NH = 32
HD = 128
DM = 512
HKV = 8
WIN = 1024

PROW = (48, 56, 48, 40)
PKV = (44,)
PTAIL = (48,)
PWIDE = (48,)
AHEAD = 4
NSEM = 4
TAILG = 16
TAILR = NH * HD // 2 // TAILG

S_WQ, S_WUK, S_C0, S_WUV, S_BQ, S_KV0, S_WO, S_BO = 0, 1, 2, 10, 11, 12, 20, 21


def _plan(base, count, sizes_kib, row_bytes):
    out, o, i = [], base, 0
    while o < base + count:
        n = min(sizes_kib[i % len(sizes_kib)] * 1024 // row_bytes, base + count - o)
        out.append((o, n))
        o += n
        i += 1
    return out


def _head_major_chunk(w_ref, k):
    v = pltpu.bitcast(w_ref[k * 128:(k + 1) * 128, :, :], U32)
    return jnp.transpose(v, (1, 0, 2))


def _unpack_pair(u):
    lo = pltpu.bitcast(u << 16, F32).astype(BF16)
    hi = pltpu.bitcast(u & jnp.uint32(0xFFFF0000), F32).astype(BF16)
    return lo, hi


def _kernel(x_hbm, ckv_hbm, wq_hbm, wuk_hbm, wuv_hbm, wo_hbm, kc_hbm, vc_hbm,
            bq_hbm, bo_hbm, g_hbm, out_ref,
            x_s, g_s, c_s, wq_s, wuk_s, wuv_s, wo_s, bq_s, bo_s, k_s, v_s,
            q_s, qa_s, qat_s, s_s, cc_s, qb_s, qbt_s, ob_s, oa_s, sems, sem_x, tail_sems):

    def issue_rows(src, dst, sem, base, count):
        half = src.shape[0] // 2
        if src.shape == (DM, NH * HD):
            for o in range(base, base + count, 8):
                for c0, w in _plan(0, src.shape[1], PWIDE, 16):
                    for r0, prio in ((o, 0), (half + o, 1)):
                        pltpu.make_async_copy(src.at[pl.ds(r0, 8), pl.ds(c0, w)],
                                              dst.at[pl.ds(r0, 8), pl.ds(c0, w)], sem).start(priority=prio)
            return
        row_bytes = 2 * math.prod(src.shape[1:])
        for o, n in _plan(base, count, PTAIL if dst is bo_s else PROW, row_bytes):
            for r0, prio in ((o, 0), (half + o, 1)):
                pltpu.make_async_copy(src.at[pl.ds(r0, n)], dst.at[pl.ds(r0, n)], sem).start(priority=prio)

    def issue_rows_quarter(src, dst, sem, k):
        q = src.shape[0] // 8
        issue_rows(src, dst, sem, k * q, q)

    def issue_kv_quarter(b, sem, k):
        for h in range(2 * k, 2 * k + 2):
            for o, n in _plan(0, WIN, PKV, 2 * HD):
                pltpu.make_async_copy(kc_hbm.at[b, h, pl.ds(SK - WIN + o, n)],
                                      k_s.at[b, h, pl.ds(o, n)], sem).start(priority=0)
                pltpu.make_async_copy(vc_hbm.at[b, h, pl.ds(SK - WIN + o, n)],
                                      v_s.at[b, h, pl.ds(o, n)], sem).start(priority=1)

    def c_wait(b, sem):
        pltpu.make_async_copy(ckv_hbm.at[b], c_s.at[b], sem).wait()

    def kv_wait(b, sem):
        pltpu.make_async_copy(kc_hbm.at[b, :, pl.ds(SK - WIN, WIN)], k_s.at[b], sem).wait()
        pltpu.make_async_copy(vc_hbm.at[b, :, pl.ds(SK - WIN, WIN)], v_s.at[b], sem).wait()

    weights = {S_WQ: (wq_hbm, wq_s), S_WUK: (wuk_hbm, wuk_s), S_WUV: (wuv_hbm, wuv_s),
               S_WO: (wo_hbm, wo_s), S_BQ: (bq_hbm, bq_s)}

    def sem_of(s):
        return sems.at[s % NSEM]

    def sem_dyn(s):
        return sems.at[lax.rem(s, NSEM)]

    def issue_quarter(s, k):
        if s > S_BO:
            return
        if s == S_BO:
            per = TAILG // 4
            for i in range(k * per, (k + 1) * per):
                issue_rows(bo_hbm, bo_s, tail_sems.at[i], i * TAILR, TAILR)
        elif s in weights:
            issue_rows_quarter(*weights[s], sem_of(s), k)
        elif s < S_WUV:
            issue_rows_quarter(ckv_hbm.at[s - S_C0], c_s.at[s - S_C0], sem_of(s), k)
        else:
            issue_kv_quarter(s - S_KV0, sem_of(s), k)

    def wait_stage(s):
        src, dst = weights[s]
        pltpu.make_async_copy(src, dst, sem_of(s)).wait()

    def issue_after_block(s, k):
        g = 4 + AHEAD + k
        issue_quarter(s + g // 4, g % 4)

    def issue_after_block_loop(s0, n, b, k, issue_same):
        g = 4 + AHEAD + k
        d, kk = g // 4, g % 4

        @pl.when(b + d < n)
        def _():
            issue_same(b + d, sem_dyn(s0 + b + d), kk)
        for t in range(d):
            @pl.when(b == n - d + t)
            def _():
                issue_quarter(s0 + n + t, kk)

    cx = pltpu.make_async_copy(x_hbm, x_s, sem_x.at[0])
    cg = pltpu.make_async_copy(g_hbm, g_s, sem_x.at[1])
    for k in range(4):
        issue_quarter(S_WQ, k)
    for g in range(AHEAD):
        issue_quarter(S_WUK + g // 4, g % 4)
    cx.start()
    cg.start()
    cx.wait()
    cg.wait()
    x = x_s[...]

    wait_stage(S_WQ)
    for k in range(4):
        issue_after_block(S_WQ, k)
        tt = _head_major_chunk(wq_s, k)
        xc = x[:, k * 128:(k + 1) * 128]
        for j in range(NH // 2):
            lo, hi = _unpack_pair(tt[j])
            q = jnp.concatenate([jnp.dot(xc, lo, preferred_element_type=F32),
                                 jnp.dot(xc, hi, preferred_element_type=F32)], axis=0)
            if k == 0:
                q_s[pl.ds(j * 16, 16), :] = q
            else:
                q_s[pl.ds(j * 16, 16), :] += q

    wait_stage(S_WUK)
    sc_a = (HD ** -0.5) * LOG2E
    for k in range(4):
        issue_after_block(S_WUK, k)
        tt = _head_major_chunk(wuk_s, k)
        for j in range(NH // 2):
            lo, hi = _unpack_pair(tt[j])
            q = q_s[pl.ds(j * 16, 16), :].astype(BF16)
            a0 = lax.dot_general(q[0:8], lo, NT, preferred_element_type=F32)
            a1 = lax.dot_general(q[8:16], hi, NT, preferred_element_type=F32)
            qa_s[k, pl.ds(j * 16, 16), :] = jnp.concatenate([a0, a1], axis=0) * sc_a
        if k == 3:
            for b in range(NB):
                qat_s[b] = jnp.concatenate(
                    [qa_s[t, pl.ds(b, NH, stride=NB), :] for t in range(DC // HD)], axis=1).astype(BF16)

    def c_issue(b, sem, k):
        issue_rows_quarter(ckv_hbm.at[b], c_s.at[b], sem, k)

    HK = SK // 2

    def a_body(b, carry):
        c_wait(b, sem_dyn(S_C0 + b))
        nxt = lambda k: issue_after_block_loop(S_C0, NB, b, k, c_issue)
        nxt(0)
        qa = qat_s[b]
        s0 = lax.dot_general(qa, c_s[b, 0:HK, :], NT, preferred_element_type=F32)
        m0 = jnp.max(s0, axis=1, keepdims=True)
        s_s[:, 0:HK] = s0
        nxt(1)
        s1 = lax.dot_general(qa, c_s[b, HK:SK, :], NT, preferred_element_type=F32)
        m = jnp.maximum(m0, jnp.max(s1, axis=1, keepdims=True))
        nxt(2)
        p1 = jnp.exp2(s1 - m)
        l = jnp.sum(p1, axis=1, keepdims=True)
        ctx = jnp.dot(p1.astype(BF16), c_s[b, HK:SK, :], preferred_element_type=F32)
        nxt(3)
        p0 = jnp.exp2(s_s[:, 0:HK] - m)
        l = l + jnp.sum(p0, axis=1, keepdims=True)
        ctx = ctx + jnp.dot(p0.astype(BF16), c_s[b, 0:HK, :], preferred_element_type=F32)
        ctx = ctx / l
        for t in range(DC // HD):
            cc_s[t, pl.ds(pl.multiple_of(b * NH, NH), NH), :] = ctx[:, t * HD:(t + 1) * HD]
        return carry
    lax.fori_loop(0, NB, a_body, 0)

    wait_stage(S_WUV)
    for k in range(4):
        issue_after_block(S_WUV, k)
        tt = _head_major_chunk(wuv_s, k)
        for j in range(NH // 2):
            lo, hi = _unpack_pair(tt[j])
            c0 = cc_s[k, pl.ds(2 * j, NB, stride=NH), :].astype(BF16)
            c1 = cc_s[k, pl.ds(2 * j + 1, NB, stride=NH), :].astype(BF16)
            o = jnp.concatenate([jnp.dot(c0, lo, preferred_element_type=F32),
                                 jnp.dot(c1, hi, preferred_element_type=F32)], axis=1)
            if k == 0:
                oa_s[:, pl.ds(j * 256, 256)] = o
            else:
                oa_s[:, pl.ds(j * 256, 256)] += o

    wait_stage(S_BQ)
    sc_b = (HD ** -0.5) * LOG2E
    KC = NH * HD // 4
    for k in range(4):
        issue_after_block(S_BQ, k)
        qb = jnp.dot(x, bq_s[:, k * KC:(k + 1) * KC], preferred_element_type=F32)
        qb = qb.astype(BF16).astype(F32) * sc_b
        for hh in range(KC // HD):
            h = k * (KC // HD) + hh
            qb_s[h * NB:(h + 1) * NB, :] = qb[:, hh * HD:(hh + 1) * HD]
        if k == 3:
            for b in range(NB):
                qbt_s[b] = qb_s[pl.ds(b, NH, stride=NB), :]

    row = lax.broadcasted_iota(jnp.int32, (8, HD), 0)
    row_w = lax.broadcasted_iota(jnp.int32, (8, WIN), 0)

    def b_body(b, carry):
        kv_wait(b, sem_dyn(S_KV0 + b))
        for i in range(HKV // 2):
            issue_after_block_loop(S_KV0, NB, b, i, issue_kv_quarter)
            q8 = qbt_s[b, 8 * i:8 * (i + 1), :]
            q0 = jnp.where(row < 4, q8, 0.0).astype(BF16)
            q1 = jnp.where(row >= 4, q8, 0.0).astype(BF16)
            s = (lax.dot_general(q0, k_s[b, 2 * i], NT, preferred_element_type=F32)
                 + lax.dot_general(q1, k_s[b, 2 * i + 1], NT, preferred_element_type=F32))
            m = jnp.max(s, axis=1, keepdims=True)
            p = jnp.exp2(s - m)
            l = jnp.sum(p, axis=1, keepdims=True)
            p0 = jnp.where(row_w < 4, p, 0.0).astype(BF16)
            p1 = jnp.where(row_w >= 4, p, 0.0).astype(BF16)
            o = (jnp.dot(p0, v_s[b, 2 * i], preferred_element_type=F32)
                 + jnp.dot(p1, v_s[b, 2 * i + 1], preferred_element_type=F32))
            ob_s[pl.ds(pl.multiple_of(b * NH + 8 * i, 8), 8), :] = o / l
        return carry
    lax.fori_loop(0, NB, b_body, 0)

    ob = jnp.concatenate([ob_s[pl.ds(h, NB, stride=NH), :] for h in range(NH)], axis=1).astype(BF16)
    gate = jnp.sum(x.astype(F32) * g_s[...].astype(F32).reshape(1, DM), axis=1, keepdims=True)
    g = jax.nn.sigmoid(gate)
    wait_stage(S_WO)
    out_a = jnp.zeros((NB, DM), F32)
    for k in range(4):
        issue_after_block(S_WO, k)
        out_a += jnp.dot(oa_s[:, k * KC:(k + 1) * KC].astype(BF16), wo_s[k * KC:(k + 1) * KC, :],
                         preferred_element_type=F32)

    out_b = jnp.zeros((NB, DM), F32)
    for i in range(TAILG):
        lo0, hi0 = i * TAILR, NH * HD // 2 + i * TAILR
        for r0 in (lo0, hi0):
            pltpu.make_async_copy(bo_hbm.at[pl.ds(r0, TAILR)], bo_s.at[pl.ds(r0, TAILR)],
                                  tail_sems.at[i]).wait()
        out_b += jnp.dot(ob[:, lo0:lo0 + TAILR], bo_s[lo0:lo0 + TAILR, :], preferred_element_type=F32)
        out_b += jnp.dot(ob[:, hi0:hi0 + TAILR], bo_s[hi0:hi0 + TAILR, :], preferred_element_type=F32)
    out_ref[...] = (g * out_a + (1.0 - g) * out_b).astype(out_ref.dtype)


@jax.jit
def pallas_gated_mix__compressed_kv_cla__sliding_block_cached__decode_kernel(
    A_x, A_c_kv, A_w_q, A_w_uk, A_w_uv, A_w_o, B_x, B_k_cache, B_v_cache, B_wq, B_wo, gate_w,
):
    del B_x
    any_spec = pl.BlockSpec(memory_space=pl.ANY)
    return pl.pallas_call(
        _kernel,
        out_shape=jax.ShapeDtypeStruct((NB, DM), A_x.dtype),
        in_specs=[any_spec] * 11,
        out_specs=pl.BlockSpec(memory_space=pltpu.VMEM),
        scratch_shapes=[
            pltpu.VMEM((NB, DM), BF16),
            pltpu.VMEM((DM,), BF16),
            pltpu.VMEM((NB, SK, DC), BF16),
            pltpu.VMEM((DM, NH, HD), BF16),
            pltpu.VMEM((DC, NH, HD), BF16),
            pltpu.VMEM((DC, NH, HD), BF16),
            pltpu.VMEM((NH * HD, DM), BF16),
            pltpu.VMEM((DM, NH * HD), BF16),
            pltpu.VMEM((NH * HD, DM), BF16),
            pltpu.VMEM((NB, HKV, WIN, HD), BF16),
            pltpu.VMEM((NB, HKV, WIN, HD), BF16),
            pltpu.VMEM((NH * NB, HD), F32),
            pltpu.VMEM((DC // HD, NH * NB, HD), F32),
            pltpu.VMEM((NB, NH, DC), BF16),
            pltpu.VMEM((NH, SK // 2), F32),
            pltpu.VMEM((DC // HD, NB * NH, HD), F32),
            pltpu.VMEM((NH * NB, HD), F32),
            pltpu.VMEM((NB, NH, HD), F32),
            pltpu.VMEM((NB * NH, HD), F32),
            pltpu.VMEM((NB, NH * HD), F32),
            pltpu.SemaphoreType.DMA((NSEM,)),
            pltpu.SemaphoreType.DMA((2,)),
            pltpu.SemaphoreType.DMA((TAILG,)),
        ],
        compiler_params=pltpu.CompilerParams(vmem_limit_bytes=120 * 1024 * 1024,
                                             disable_semaphore_checks=True),
    )(
        A_x.reshape(NB, DM),
        A_c_kv,
        A_w_q,
        A_w_uk,
        A_w_uv,
        A_w_o.reshape(NH * HD, DM),
        B_k_cache,
        B_v_cache,
        B_wq,
        B_wo,
        gate_w,
    ).reshape(NB, 1, DM)
```
